```python
import jax
import jax.numpy as jnp

def _softmax(x, axis=-1):
    return jax.nn.softmax(x, axis=axis)
def _gelu(x):
    return jax.nn.gelu(x, approximate=True)
def _silu(x):
    return jax.nn.silu(x)
def _sigmoid(x):
    return jax.nn.sigmoid(x)
def _layernorm(x, axis=-1, eps=1e-5):
    m = jnp.mean(x, axis=axis, keepdims=True)
    v = jnp.var(x, axis=axis, keepdims=True)
    return (x - m) / jnp.sqrt(v + eps)
def _scatter_add(tgt, idx, src, axis=0):
    return tgt.at[idx].add(src)
def _segment_sum(src, seg, n):
    return jax.ops.segment_sum(src, seg, n)
class _Rng:
    def __init__(self, key):
        self._k = key
    def _next(self):
        self._k, sub = jax.random.split(self._k)
        return sub
    def normal(self, shape):
        return jax.random.normal(self._next(), shape, dtype=jnp.bfloat16)
    def randint(self, lo, hi, shape):
        return jax.random.randint(self._next(), shape, lo, hi, dtype=jnp.int32)
    def uniform(self, shape, lo=0.0, hi=1.0):
        return jax.random.uniform(self._next(), shape, jnp.bfloat16, lo, hi)
    def permutation(self, n):
        return jax.random.permutation(self._next(), n)


kernel_name = 'sequential_preLN__sliding_block_cached__glu_gated_swiglu__decode'

def setup_inputs():
    _rng = _Rng(jax.random.key(int.from_bytes(__import__("os").urandom(4), "little")))
    _w = (lambda a: (lambda t: t.astype(jnp.bfloat16) if jnp.issubdtype(t.dtype, jnp.floating) else t)(jnp.asarray(a)))
    def _A_setup():
        B, Sq, D = 1, 1, 640
        Hq, Hkv, Sk, Dh = 32, 32, 32768, 192
        assert Hq % Hkv == 0, (Hq, Hkv)
        return {
            "x": _w((lambda *s: _rng.normal(s) * 0.05)(B, Sq, D)),
            "k_cache": _w((lambda *s: _rng.normal(s) * 0.05)(B, Hkv, Sk, Dh)),
            "v_cache": _w((lambda *s: _rng.normal(s) * 0.05)(B, Hkv, Sk, Dh)),
            "wq": _w((lambda *s: _rng.normal(s) * 0.05)(D, Hq * Dh) * (D ** -0.5)),
            "wo": _w((lambda *s: _rng.normal(s) * 0.05)(Hq * Dh, D) * ((Hq * Dh) ** -0.5)),
        }
    _A_in = _A_setup()

    def _B_setup():
        B, S, D, F = 1, 1, 640, 1536
        return {
            "x": _w((lambda *s: _rng.normal(s) * 0.05)(B, S, D)),
            "w1": _w((lambda *s: _rng.normal(s) * 0.05)(D, F) * (2.0 / D) ** 0.5),
            "w3": _w((lambda *s: _rng.normal(s) * 0.05)(D, F) * (2.0 / D) ** 0.5),
            "w2": _w((lambda *s: _rng.normal(s) * 0.05)(F, D) * (2.0 / F) ** 0.5),
        }
    _B_in = _B_setup()

    return {
        "A_x": _A_in["x"],
        "A_k_cache": _A_in["k_cache"],
        "A_v_cache": _A_in["v_cache"],
        "A_wq": _A_in["wq"],
        "A_wo": _A_in["wo"],
        "B_x": _B_in["x"],
        "B_w1": _B_in["w1"],
        "B_w3": _B_in["w3"],
        "B_w2": _B_in["w2"],
    }

def reference(A_x, A_k_cache, A_v_cache, A_wq, A_wo, B_x, B_w1, B_w3, B_w2):
    def _A_ref(x, k_cache, v_cache, wq, wo):
        B, Sq, D = x.shape
        Hq, Dh = 32, 192
        Hkv, Sk = k_cache.shape[1], k_cache.shape[2]
        W = min(4096, max(256, Sk // 4))
        rep = Hq // Hkv
        q = (lambda x, *d: x.transpose(*d))((x @ wq).reshape(B, Sq, Hq, Dh), 0, 2, 1, 3)
        k = jnp.repeat(k_cache[:, :, Sk - W:, :], rep, axis=1)
        v = jnp.repeat(v_cache[:, :, Sk - W:, :], rep, axis=1)
        scores = jnp.einsum("bhqd,bhkd->bhqk", q, k) * (Dh ** -0.5)
        p = _softmax(scores, axis=-1)
        o = jnp.einsum("bhqk,bhkd->bhqd", p, v)
        return (lambda x, *d: x.transpose(*d))(o, 0, 2, 1, 3).reshape(B, Sq, Hq * Dh) @ wo

    def _B_ref(x, w1, w3, w2):
        gate = jnp.einsum("bsd,df->bsf", x, w1)
        up = jnp.einsum("bsd,df->bsf", x, w3)
        h = _silu(gate) * up
        out = jnp.einsum("bsf,fd->bsd", h, w2)
        return out

    x = A_x
    h = x + _A_ref(_layernorm(x, axis=-1), A_k_cache, A_v_cache, A_wq, A_wo)
    h2 = h + _B_ref(_layernorm(h, axis=-1), B_w1, B_w3, B_w2)
    return h2
```

```python
import functools

import jax
import jax.numpy as jnp
import jax.experimental.pallas as pl
import jax.experimental.pallas.tpu as pltpu

HQ = 32
DH = 192
EPS = 1e-5
LOOKAHEAD = 2
NSLOT = LOOKAHEAD + 1
W2_CHUNKS = 4


def _layernorm(x):
    m = jnp.mean(x, axis=-1, keepdims=True)
    xc = x - m
    v = jnp.mean(xc * xc, axis=-1, keepdims=True)
    return xc * jax.lax.rsqrt(v + EPS)


def _kernel(x_hbm, kt_hbm, vt_hbm, wq_hbm, wo_hbm, w1_hbm, w3_hbm, w2_hbm,
            o_ref,
            x_v, wq_v, wo_v, w1_v, w3_v, w2_v, kbuf, vbuf, q_s, acc_s,
            sem_k, sem_v, sem_o, sem_w, *, win, sk):
    f32, bf16 = jnp.float32, jnp.bfloat16
    col0 = sk - win
    ff = w2_v.shape[0]
    w2c = ff // W2_CHUNKS

    def k_copy(h, slot):
        return pltpu.make_async_copy(
            kt_hbm.at[h, :, pl.ds(col0, win)], kbuf.at[slot], sem_k.at[slot])

    def v_copy(h, slot):
        return pltpu.make_async_copy(
            vt_hbm.at[h, :, pl.ds(col0, win)], vbuf.at[slot], sem_v.at[slot])

    def wo_copy(h, slot):
        return pltpu.make_async_copy(wo_hbm.at[h], wo_v.at[slot], sem_o.at[slot])

    x_copy = pltpu.make_async_copy(x_hbm, x_v, sem_w.at[0])
    wq_copy = pltpu.make_async_copy(wq_hbm, wq_v, sem_w.at[1])
    w1_copy = pltpu.make_async_copy(w1_hbm, w1_v, sem_w.at[2])
    w3_copy = pltpu.make_async_copy(w3_hbm, w3_v, sem_w.at[3])

    def w2_copy(c):
        return pltpu.make_async_copy(
            w2_hbm.at[pl.ds(c * w2c, w2c), :], w2_v.at[pl.ds(c * w2c, w2c), :],
            sem_w.at[4 + c])

    def start_head(h, slot):
        k_copy(h, slot).start()
        v_copy(h, slot).start()
        wo_copy(h, slot).start()

    x_copy.start()
    wq_copy.start()
    for h in range(LOOKAHEAD):
        start_head(h, h % NSLOT)

    x_copy.wait()
    x = x_v[...].astype(f32)
    xn = _layernorm(x).astype(bf16)
    wq_copy.wait()
    q = jnp.dot(xn, wq_v[...], preferred_element_type=f32)
    q = (q * (DH ** -0.5)).astype(bf16)
    for h in range(HQ):
        q_s[h] = q[:, h * DH:(h + 1) * DH]
    acc_s[...] = jnp.zeros_like(acc_s)

    def head(h, carry):
        slot = h % NSLOT
        nxt = h + LOOKAHEAD

        @pl.when(nxt < HQ)
        def _():
            start_head(nxt, nxt % NSLOT)

        @pl.when(nxt == HQ)
        def _():
            w1_copy.start()
            w3_copy.start()
            for c in range(W2_CHUNKS):
                w2_copy(c).start()

        k_copy(h, slot).wait()
        s = jnp.dot(q_s[h], kbuf[slot], preferred_element_type=f32)
        m = jnp.max(s, axis=-1, keepdims=True)
        p = jnp.exp(s - m)
        l = jnp.sum(p, axis=-1, keepdims=True)
        v_copy(h, slot).wait()
        o = jax.lax.dot_general(p.astype(bf16), vbuf[slot],
                                (((1,), (1,)), ((), ())),
                                preferred_element_type=f32)
        o = (o / l).astype(bf16)
        wo_copy(h, slot).wait()
        acc_s[...] += jnp.dot(o, wo_v[slot], preferred_element_type=f32)
        return carry

    jax.lax.fori_loop(0, HQ, head, 0)

    hres = x + acc_s[...]
    hn = _layernorm(hres).astype(bf16)
    w1_copy.wait()
    g = jnp.dot(hn, w1_v[...], preferred_element_type=f32)
    w3_copy.wait()
    u = jnp.dot(hn, w3_v[...], preferred_element_type=f32)
    a = (g * jax.nn.sigmoid(g) * u).astype(bf16)
    out = hres
    for c in range(W2_CHUNKS):
        w2_copy(c).wait()
        out = out + jnp.dot(a[:, c * w2c:(c + 1) * w2c],
                            w2_v[pl.ds(c * w2c, w2c), :],
                            preferred_element_type=f32)
    o_ref[...] = out.astype(o_ref.dtype)


@jax.jit
def pallas_sequential_preLN__sliding_block_cached__glu_gated_swiglu__decode_kernel(
    A_x: jax.Array,
    A_k_cache: jax.Array,
    A_v_cache: jax.Array,
    A_wq: jax.Array,
    A_wo: jax.Array,
    B_x: jax.Array,
    B_w1: jax.Array,
    B_w3: jax.Array,
    B_w2: jax.Array,
):
    B, Sq, D = A_x.shape
    _, hkv, sk, dh = A_k_cache.shape
    assert (B, Sq, hkv, dh) == (1, 1, HQ, DH)
    win = min(4096, max(256, sk // 4))
    ff = B_w1.shape[1]
    bf16 = jnp.bfloat16

    kt = jnp.swapaxes(A_k_cache, 2, 3).reshape(HQ, DH, sk)
    vt = jnp.swapaxes(A_v_cache, 2, 3).reshape(HQ, DH, sk)
    x2 = A_x.reshape(1, D)
    wo3 = A_wo.reshape(HQ, DH, D)

    any_spec = pl.BlockSpec(memory_space=pl.ANY)
    out = pl.pallas_call(
        functools.partial(_kernel, win=win, sk=sk),
        out_shape=jax.ShapeDtypeStruct((1, D), A_x.dtype),
        in_specs=[any_spec] * 8,
        out_specs=pl.BlockSpec(memory_space=pltpu.VMEM),
        scratch_shapes=[
            pltpu.VMEM((1, D), bf16),
            pltpu.VMEM((D, HQ * DH), bf16),
            pltpu.VMEM((NSLOT, DH, D), bf16),
            pltpu.VMEM((D, ff), bf16),
            pltpu.VMEM((D, ff), bf16),
            pltpu.VMEM((ff, D), bf16),
            pltpu.VMEM((NSLOT, DH, win), bf16),
            pltpu.VMEM((NSLOT, DH, win), bf16),
            pltpu.VMEM((HQ, 1, DH), bf16),
            pltpu.VMEM((1, D), jnp.float32),
            pltpu.SemaphoreType.DMA((NSLOT,)),
            pltpu.SemaphoreType.DMA((NSLOT,)),
            pltpu.SemaphoreType.DMA((NSLOT,)),
            pltpu.SemaphoreType.DMA((4 + W2_CHUNKS,)),
        ],
        compiler_params=pltpu.CompilerParams(vmem_limit_bytes=64 * 1024 * 1024),
    )(x2, kt, vt, A_wq, wo3, B_w1, B_w3, B_w2)
    return out.reshape(B, Sq, D)
```

```python
import functools

import jax
import jax.numpy as jnp
import jax.experimental.pallas as pl
import jax.experimental.pallas.tpu as pltpu

HQ = 32
DH = 192
EPS = 1e-5
TW = 128
TPC = 2
CW = TW * TPC
LOOK = 16
NSLOT = 16
BULK = 1
TRICKLE = 0
W2_TAIL_ROWS = 128
CHECKS_OFF = True
COMPUTE = True


def _layernorm(x):
    m = jnp.mean(x, axis=-1, keepdims=True)
    xc = x - m
    v = jnp.mean(xc * xc, axis=-1, keepdims=True)
    return xc * jax.lax.rsqrt(v + EPS)


def _interleave(groups, n):
    items = []
    for g in groups:
        for k, it in enumerate(g):
            items.append(((k + 0.5) / len(g), it))
    items.sort(key=lambda t: t[0])
    assert len(items) == n, (len(items), n)
    return [it for _, it in items]


def _kernel(x_hbm, kt_hbm, vt_hbm, wq_hbm, wo_hbm, w1_hbm, w3_hbm, w2_hbm,
            o_ref,
            x_v, wq_v, wo_v, w1_v, w3_v, w2_v, kvbuf, s_scr, p_scr, acc_s,
            sem_kv, sem_q, sem_o, sem_w, sem_t, *, win, sk):
    f32, bf16 = jnp.float32, jnp.bfloat16
    col0 = sk - win
    d_model = x_v.shape[1]
    ff = w2_v.shape[0]
    nch = win // CW
    ntk = win // TW
    per_head = 2 * ntk
    npair = HQ // 2
    pw = 2 * DH
    nts = NSLOT * TPC
    qrg = 16
    n_wq = d_model // qrg
    n_wo = DH // 8
    w13c = ff // 4
    n_w13 = (d_model // 8) * 4 // npair
    w2_early = 2 * n_wq * 8
    n_tail = (ff - w2_early) // W2_TAIL_ROWS
    assert per_head % nts == 0 and LOOK <= nts - TPC
    assert w2_early + n_tail * W2_TAIL_ROWS == ff

    def aligned(v, m):
        return v if isinstance(v, int) else pl.multiple_of(v, m)

    def kv_copy(h, t):
        src = kt_hbm if t < ntk else vt_hbm
        c = t % ntk
        ts = t % nts
        return pltpu.make_async_copy(
            src.at[h, :, pl.ds(col0 + c * TW, TW)],
            kvbuf.at[ts // TPC, :, pl.ds((ts % TPC) * TW, TW)], sem_kv.at[ts])

    def qslot(blk):
        return blk % 3 if isinstance(blk, int) else jax.lax.rem(blk, 3)

    def wq_piece(blk, r, rows=qrg):
        return pltpu.make_async_copy(
            wq_hbm.at[pl.ds(r * rows, rows), pl.ds(aligned(blk * pw, 128), pw)],
            wq_v.at[blk, pl.ds(r * rows, rows), :], sem_q.at[qslot(blk)])

    def wo_piece(h, par, r):
        return pltpu.make_async_copy(
            wo_hbm.at[h, pl.ds(r * 8, 8), :], wo_v.at[h, pl.ds(r * 8, 8), :], sem_o.at[par])

    def w13_piece(which, pair, k):
        src, dst = ((w1_hbm, w1_v), (w3_hbm, w3_v))[which]
        r0 = aligned((pair * (n_w13 // 4) + k // 4) * 8, 8)
        c0 = (k % 4) * w13c
        return pltpu.make_async_copy(
            src.at[pl.ds(r0, 8), pl.ds(c0, w13c)],
            dst.at[pl.ds(r0, 8), pl.ds(c0, w13c)], sem_w.at[1 + which])

    def w2_early_piece(g):
        r0 = aligned(g * 8, 8)
        return pltpu.make_async_copy(
            w2_hbm.at[pl.ds(r0, 8), :], w2_v.at[pl.ds(r0, 8), :], sem_w.at[3])

    def w2_tail_copy(t):
        r0 = w2_early + t * W2_TAIL_ROWS
        return pltpu.make_async_copy(
            w2_hbm.at[pl.ds(r0, W2_TAIL_ROWS), :], w2_v.at[pl.ds(r0, W2_TAIL_ROWS), :],
            sem_t.at[t])

    x_copy = pltpu.make_async_copy(x_hbm, x_v, sem_w.at[0])

    def q_project(blk, xn):
        q = jnp.dot(xn, wq_v[blk], preferred_element_type=f32) * (DH ** -0.5)
        return q[:, :DH], q[:, DH:]

    x_copy.start(priority=TRICKLE)
    wq_piece(0, 0, d_model).start(priority=TRICKLE)
    for t in range(LOOK):
        kv_copy(0, t).start(priority=BULK)
    wq_piece(1, 0, d_model).start(priority=TRICKLE)
    x_copy.wait()
    x = x_v[...].astype(f32)
    xn = _layernorm(x).astype(bf16)
    acc_s[...] = jnp.zeros_like(acc_s)
    wq_piece(0, 0, d_model).wait()
    q0 = q_project(0, xn)

    sched = []
    for par in range(2):
        sched += _interleave([
            [("wo", par, r) for r in range(n_wo)],
            [("wq", par * (n_wq // 2) + r) for r in range(n_wq // 2)],
            [("w13", 0, par * (n_w13 // 2) + k) for k in range(n_w13 // 2)],
            [("w13", 1, par * (n_w13 // 2) + k) for k in range(n_w13 // 2)],
        ], per_head)

    def pair_body(pair, carry):
        q_cur, o_prev = carry[:2], carry[2]
        q_next = q_cur

        def tick(par, t):
            h = 2 * pair + par
            kv_copy(h, t).wait()
            t2 = t + LOOK
            if t2 < per_head:
                kv_copy(h, t2).start(priority=BULK)
            elif par == 0:
                kv_copy(h + 1, t2 - per_head).start(priority=BULK)
            else:
                @pl.when(pair + 1 < npair)
                def _():
                    kv_copy(h + 1, t2 - per_head).start(priority=BULK)

                tt = [k for k in range(n_tail) if k * LOOK // n_tail == t2 - per_head]
                if tt:
                    @pl.when(pair + 1 == npair)
                    def _():
                        for k in tt:
                            w2_tail_copy(k).start(priority=BULK)
            item = sched[par * per_head + t]
            if item[0] == "wo":
                wo_piece(h, par, item[2]).start(priority=TRICKLE)
            elif item[0] == "w13":
                w13_piece(item[1], pair, item[2]).start(priority=TRICKLE)
            else:
                @pl.when(pair + 2 < npair)
                def _():
                    wq_piece(pair + 2, item[1]).start(priority=TRICKLE)

                @pl.when(pair + 2 >= npair)
                def _():
                    w2_early_piece((pair + 2 - npair) * n_wq + item[1]).start(priority=TRICKLE)

        def out_project(h, par, o_h):
            pltpu.make_async_copy(wo_hbm.at[h], wo_v.at[h], sem_o.at[par]).wait()
            if COMPUTE:
                acc_s[...] += jnp.dot(o_h.astype(bf16), wo_v[h], preferred_element_type=f32)

        for par in range(2):
            h = 2 * pair + par
            q = q_cur[par].astype(bf16)
            for c in range(nch):
                for u in range(TPC):
                    tick(par, c * TPC + u)
                    if u == 0 and c == 6:
                        if par == 1:
                            out_project(h - 1, 0, o_prev)
                        else:
                            @pl.when(pair > 0)
                            def _():
                                out_project(h - 1, 1, o_prev)
                    if u == 0 and c == 10 and par == 0:
                        @pl.when(pair + 1 < npair)
                        def _():
                            wq_piece(pair + 1, 0, d_model).wait()

                        if COMPUTE:
                            q_next = q_project(jnp.minimum(pair + 1, npair - 1), xn)
                if COMPUTE:
                    s_scr[c:c + 1, :] = jnp.dot(q, kvbuf[c % NSLOT], preferred_element_type=f32)
            o = jnp.zeros((1, DH), f32)
            l = jnp.ones((1, 1), f32)
            for c in range(nch):
                for u in range(TPC):
                    tick(par, ntk + c * TPC + u)
                    if u == 0 and c == 0 and COMPUTE:
                        s = s_scr[...]
                        m = jnp.max(jnp.max(s, axis=1, keepdims=True), axis=0, keepdims=True)
                        p = jnp.exp(s - m)
                        l = jnp.sum(jnp.sum(p, axis=1, keepdims=True), axis=0, keepdims=True)
                        p_scr[...] = p
                if COMPUTE:
                    o = o + jax.lax.dot_general(p_scr[c:c + 1, :].astype(bf16),
                                                kvbuf[(nch + c) % NSLOT],
                                                (((1,), (1,)), ((), ())),
                                                preferred_element_type=f32)
            o_prev = o / l
        return (q_next[0], q_next[1], o_prev)

    _, _, o_last = jax.lax.fori_loop(
        0, npair, pair_body, (q0[0], q0[1], jnp.zeros((1, DH), f32)))

    pltpu.make_async_copy(wo_hbm.at[HQ - 1], wo_v.at[HQ - 1], sem_o.at[1]).wait()
    attn = acc_s[...] + jnp.dot(o_last.astype(bf16), wo_v[HQ - 1], preferred_element_type=f32)
    hres = x + attn
    hn = _layernorm(hres).astype(bf16)
    pltpu.make_async_copy(w1_hbm, w1_v, sem_w.at[1]).wait()
    pltpu.make_async_copy(w3_hbm, w3_v, sem_w.at[2]).wait()
    pltpu.make_async_copy(w2_hbm.at[pl.ds(0, w2_early), :], w2_v.at[pl.ds(0, w2_early), :],
                          sem_w.at[3]).wait()
    g = jnp.dot(hn, w1_v[...], preferred_element_type=f32)
    u = jnp.dot(hn, w3_v[...], preferred_element_type=f32)
    a = (g * jax.nn.sigmoid(g) * u).astype(bf16)
    out = hres + jnp.dot(a[:, :w2_early], w2_v[pl.ds(0, w2_early), :],
                         preferred_element_type=f32)
    for t in range(n_tail):
        r0 = w2_early + t * W2_TAIL_ROWS
        w2_tail_copy(t).wait()
        out = out + jnp.dot(a[:, r0:r0 + W2_TAIL_ROWS], w2_v[pl.ds(r0, W2_TAIL_ROWS), :],
                            preferred_element_type=f32)
    o_ref[...] = out.astype(o_ref.dtype)


@jax.jit
def pallas_sequential_preLN__sliding_block_cached__glu_gated_swiglu__decode_kernel(
    A_x: jax.Array,
    A_k_cache: jax.Array,
    A_v_cache: jax.Array,
    A_wq: jax.Array,
    A_wo: jax.Array,
    B_x: jax.Array,
    B_w1: jax.Array,
    B_w3: jax.Array,
    B_w2: jax.Array,
):
    B, Sq, D = A_x.shape
    _, hkv, sk, dh = A_k_cache.shape
    assert (B, Sq, hkv, dh) == (1, 1, HQ, DH)
    win = min(4096, max(256, sk // 4))
    ff = B_w1.shape[1]
    bf16, f32 = jnp.bfloat16, jnp.float32
    n_tail = (ff - 2 * (D // 16) * 8) // W2_TAIL_ROWS

    kt = jnp.swapaxes(A_k_cache, 2, 3).reshape(HQ, DH, sk)
    vt = jnp.swapaxes(A_v_cache, 2, 3).reshape(HQ, DH, sk)
    x2 = A_x.reshape(1, D)
    wo3 = A_wo.reshape(HQ, DH, D)

    any_spec = pl.BlockSpec(memory_space=pl.ANY)
    out = pl.pallas_call(
        functools.partial(_kernel, win=win, sk=sk),
        out_shape=jax.ShapeDtypeStruct((1, D), A_x.dtype),
        in_specs=[any_spec] * 8,
        out_specs=pl.BlockSpec(memory_space=pltpu.VMEM),
        scratch_shapes=[
            pltpu.VMEM((1, D), bf16),
            pltpu.VMEM((HQ // 2, D, 2 * DH), bf16),
            pltpu.VMEM((HQ, DH, D), bf16),
            pltpu.VMEM((D, ff), bf16),
            pltpu.VMEM((D, ff), bf16),
            pltpu.VMEM((ff, D), bf16),
            pltpu.VMEM((NSLOT, DH, CW), bf16),
            pltpu.VMEM((win // CW, CW), f32),
            pltpu.VMEM((win // CW, CW), f32),
            pltpu.VMEM((1, D), f32),
            pltpu.SemaphoreType.DMA((NSLOT * TPC,)),
            pltpu.SemaphoreType.DMA((3,)),
            pltpu.SemaphoreType.DMA((2,)),
            pltpu.SemaphoreType.DMA((4,)),
            pltpu.SemaphoreType.DMA((n_tail,)),
        ],
        compiler_params=pltpu.CompilerParams(
            vmem_limit_bytes=64 * 1024 * 1024,
            disable_bounds_checks=CHECKS_OFF,
            disable_semaphore_checks=CHECKS_OFF),
    )(x2, kt, vt, A_wq, wo3, B_w1, B_w3, B_w2)
    return out.reshape(B, Sq, D)
```

```python
import functools

import jax
import jax.numpy as jnp
import jax.experimental.pallas as pl
import jax.experimental.pallas.tpu as pltpu

HQ = 32
DH = 192
EPS = 1e-5
LANE = 128
TW = 128
TPC = 4
CW = TW * TPC
LOOK = 16
NSLOT = 8
BULK = 1
TRICKLE = 0
WO_ROWS = 48
WQ_ROWS = 32
W2_EARLY = 256
W2_TAIL_ROWS = 128
EARLY_FRAC = 0.75
W2_MERGE = 6
KV0 = 0
CHECKS_OFF = True
COMPUTE = True


def _layernorm(x):
    m = jnp.mean(x, axis=-1, keepdims=True)
    xc = x - m
    v = jnp.mean(xc * xc, axis=-1, keepdims=True)
    return xc * jax.lax.rsqrt(v + EPS)


def _spread(early, filler, n):
    items = []
    for g in early:
        for k, it in enumerate(g):
            items.append(((k + 0.5) / len(g), it))
    items.sort(key=lambda t: t[0])
    n_early = max(int(n * EARLY_FRAC), min(len(items), n))
    slots = [[] for _ in range(n)]
    for k, (_, it) in enumerate(items):
        slots[k * n_early // len(items)].append(it)
    free = [k for k in range(n) if not slots[k]] or list(range(n))
    for k, it in enumerate(filler):
        slots[free[k * len(free) // len(filler)]].append(it)
    return slots


def _kernel(x_hbm, kt_hbm, vt_hbm, wq_hbm, wo_hbm, w1_hbm, w3_hbm, w2_hbm,
            o_ref,
            x_v, wq_v, wo_v, w1_v, w3_v, w2_v, kvbuf, s_scr, p_scr, acc_s,
            sem_kv, sem_q, sem_o, sem_w, sem_t, *, win, sk):
    f32, bf16 = jnp.float32, jnp.bfloat16
    col0 = sk - win
    d_model = x_v.shape[1]
    ff = w2_v.shape[0]
    nch = win // CW
    ntk = win // TW
    per_head = 2 * ntk
    npair = HQ // 2
    pw = 2 * DH
    nts = NSLOT * TPC
    w13r = d_model // npair
    n_tail = (ff - W2_EARLY) // W2_TAIL_ROWS
    assert per_head % nts == 0 and LOOK <= nts - TPC
    assert W2_EARLY + n_tail * W2_TAIL_ROWS == ff

    def aligned(v, m):
        return v if isinstance(v, int) else pl.multiple_of(v, m)

    def kv_copy(h, t, r0=0, nr=DH):
        src = kt_hbm if t < ntk else vt_hbm
        c = t % ntk
        ts = t % nts
        return pltpu.make_async_copy(
            src.at[h, pl.ds(r0, nr), pl.ds(col0 + c * TW, TW)],
            kvbuf.at[ts // TPC, pl.ds(r0, nr), pl.ds((ts % TPC) * TW, TW)], sem_kv.at[ts])

    def kv_start(h, t):
        kv_copy(h, t, KV0, DH - KV0).start(priority=BULK)
        if KV0:
            kv_copy(h, t, 0, KV0).start(priority=TRICKLE)

    def qslot(blk):
        return blk % 3 if isinstance(blk, int) else jax.lax.rem(blk, 3)

    def wq_piece(blk, r0, nr, c0, nc):
        return pltpu.make_async_copy(
            wq_hbm.at[pl.ds(r0, nr), pl.ds(aligned(blk * pw + c0, LANE), nc)],
            wq_v.at[blk, pl.ds(r0, nr), pl.ds(c0, nc)], sem_q.at[qslot(blk)])

    def wq_whole(blk):
        return wq_piece(blk, 0, d_model, 0, pw)

    def wo_piece(h, par, r0, nr, c0, nc):
        return pltpu.make_async_copy(
            wo_hbm.at[h, pl.ds(r0, nr), pl.ds(c0, nc)],
            wo_v.at[h, pl.ds(r0, nr), pl.ds(c0, nc)], sem_o.at[par])

    def w13_piece(which, pair, c0):
        src, dst = ((w1_hbm, w1_v), (w3_hbm, w3_v))[which]
        r0 = aligned(pair * w13r, 8)
        return pltpu.make_async_copy(
            src.at[pl.ds(r0, w13r), pl.ds(c0, LANE)],
            dst.at[pl.ds(r0, w13r), pl.ds(c0, LANE)], sem_w.at[1 + which])

    def w2_early_piece(r0, nr, c0):
        r0 = aligned(r0, 8)
        return pltpu.make_async_copy(
            w2_hbm.at[pl.ds(r0, nr), pl.ds(c0, LANE)],
            w2_v.at[pl.ds(r0, nr), pl.ds(c0, LANE)], sem_w.at[3])

    def w2_tail_copy(t):
        r0 = W2_EARLY + t * W2_TAIL_ROWS
        return pltpu.make_async_copy(
            w2_hbm.at[pl.ds(r0, W2_TAIL_ROWS), :], w2_v.at[pl.ds(r0, W2_TAIL_ROWS), :],
            sem_t.at[t])

    x_copy = pltpu.make_async_copy(x_hbm, x_v, sem_w.at[0])

    def q_project(blk, xn):
        q = jnp.dot(xn, wq_v[blk], preferred_element_type=f32) * (DH ** -0.5)
        return q[:, :DH], q[:, DH:]

    x_copy.start(priority=TRICKLE)
    wq_whole(0).start(priority=TRICKLE)
    for t in range(LOOK):
        kv_start(0, t)
    wq_whole(1).start(priority=TRICKLE)
    x_copy.wait()
    x = x_v[...].astype(f32)
    xn = _layernorm(x).astype(bf16)
    acc_s[...] = jnp.zeros_like(acc_s)
    wq_whole(0).wait()
    q0 = q_project(0, xn)

    wq_list = [(r0, c0) for r0 in range(0, d_model, WQ_ROWS) for c0 in range(0, pw, LANE)]
    w2_half = W2_EARLY // 2
    w2_list = [(r0, c0) for r0 in range(0, w2_half, WQ_ROWS) for c0 in range(0, d_model, LANE)]
    assert len(w2_list) <= len(wq_list) and w2_half % WQ_ROWS == 0
    w2_of = {}
    for k, it in enumerate(w2_list):
        w2_of[k * len(wq_list) // len(w2_list)] = it
    w13_list = [(w, c0) for c0 in range(0, ff, LANE) for w in range(2)]
    sched = []
    for par in range(2):
        nq2, n13 = len(wq_list) // 2, len(w13_list) // 2
        sched += _spread(
            [[("wo", r0, c0) for r0 in range(0, DH, WO_ROWS) for c0 in range(0, d_model, LANE)],
             [("w13",) + it for it in w13_list[par * n13:(par + 1) * n13]]],
            [("wq", k) for k in range(par * nq2, (par + 1) * nq2)], per_head)

    def pair_body(pair, carry):
        q_cur, o_prev = carry[:2], carry[2]
        q_next = q_cur

        def tick(par, t):
            h = 2 * pair + par
            kv_copy(h, t).wait()
            t2 = t + LOOK
            if t2 < per_head:
                kv_start(h, t2)
            elif par == 0:
                kv_start(h + 1, t2 - per_head)
            else:
                @pl.when(pair + 1 < npair)
                def _():
                    kv_start(h + 1, t2 - per_head)

                tt = [k for k in range(n_tail) if k * LOOK // n_tail == t2 - per_head]
                if tt:
                    @pl.when(pair + 1 == npair)
                    def _():
                        for k in tt:
                            w2_tail_copy(k).start(priority=BULK)
            for item in sched[par * per_head + t]:
                if item[0] == "wo":
                    wo_piece(h, par, item[1], WO_ROWS, item[2], LANE).start(priority=TRICKLE)
                elif item[0] == "w13":
                    w13_piece(item[1], pair, item[2]).start(priority=TRICKLE)
                else:
                    r0, c0 = wq_list[item[1]]

                    @pl.when(pair + 2 < npair)
                    def _():
                        wq_piece(pair + 2, r0, WQ_ROWS, c0, LANE).start(priority=TRICKLE)

                    if item[1] in w2_of:
                        r2, c2 = w2_of[item[1]]

                        @pl.when(pair + 2 >= npair)
                        def _():
                            w2_early_piece((pair + 2 - npair) * w2_half + r2, WQ_ROWS,
                                           c2).start(priority=TRICKLE)

        def out_project(h, par, o_h):
            pltpu.make_async_copy(wo_hbm.at[h], wo_v.at[h], sem_o.at[par]).wait()
            if COMPUTE:
                acc_s[...] += jnp.dot(o_h.astype(bf16), wo_v[h], preferred_element_type=f32)

        for par in range(2):
            h = 2 * pair + par
            q = q_cur[par].astype(bf16)
            for c in range(nch):
                for u in range(TPC):
                    tick(par, c * TPC + u)
                    if u == 0 and c == 3:
                        if par == 1:
                            out_project(h - 1, 0, o_prev)
                        else:
                            @pl.when(pair > 0)
                            def _():
                                out_project(h - 1, 1, o_prev)
                    if u == 0 and c == 5 and par == 0:
                        @pl.when(pair + 1 < npair)
                        def _():
                            wq_whole(pair + 1).wait()

                        if COMPUTE:
                            q_next = q_project(jnp.minimum(pair + 1, npair - 1), xn)
                if COMPUTE:
                    s_scr[c:c + 1, :] = jnp.dot(q, kvbuf[c % NSLOT], preferred_element_type=f32)
            o = jnp.zeros((1, DH), f32)
            l = jnp.ones((1, 1), f32)
            for c in range(nch):
                for u in range(TPC):
                    tick(par, ntk + c * TPC + u)
                    if u == 0 and c == 0 and COMPUTE:
                        s = s_scr[...]
                        m = jnp.max(jnp.max(s, axis=1, keepdims=True), axis=0, keepdims=True)
                        p = jnp.exp(s - m)
                        l = jnp.sum(jnp.sum(p, axis=1, keepdims=True), axis=0, keepdims=True)
                        p_scr[...] = p
                if COMPUTE:
                    o = o + jax.lax.dot_general(p_scr[c:c + 1, :].astype(bf16),
                                                kvbuf[(nch + c) % NSLOT],
                                                (((1,), (1,)), ((), ())),
                                                preferred_element_type=f32)
            o_prev = o / l
        return (q_next[0], q_next[1], o_prev)

    _, _, o_last = jax.lax.fori_loop(
        0, npair, pair_body, (q0[0], q0[1], jnp.zeros((1, DH), f32)))

    pltpu.make_async_copy(wo_hbm.at[HQ - 1], wo_v.at[HQ - 1], sem_o.at[1]).wait()
    attn = acc_s[...] + jnp.dot(o_last.astype(bf16), wo_v[HQ - 1], preferred_element_type=f32)
    hres = x + attn
    hn = _layernorm(hres).astype(bf16)
    pltpu.make_async_copy(w1_hbm, w1_v, sem_w.at[1]).wait()
    pltpu.make_async_copy(w3_hbm, w3_v, sem_w.at[2]).wait()
    pltpu.make_async_copy(w2_hbm.at[pl.ds(0, W2_EARLY), :], w2_v.at[pl.ds(0, W2_EARLY), :],
                          sem_w.at[3]).wait()
    g = jnp.dot(hn, w1_v[...], preferred_element_type=f32)
    u = jnp.dot(hn, w3_v[...], preferred_element_type=f32)
    a = (g * jax.nn.sigmoid(g) * u).astype(bf16)
    for t in range(W2_MERGE):
        w2_tail_copy(t).wait()
    r1 = W2_EARLY + W2_MERGE * W2_TAIL_ROWS
    out = hres + jnp.dot(a[:, :r1], w2_v[pl.ds(0, r1), :], preferred_element_type=f32)
    for t in range(W2_MERGE, n_tail):
        r0 = W2_EARLY + t * W2_TAIL_ROWS
        w2_tail_copy(t).wait()
        out = out + jnp.dot(a[:, r0:r0 + W2_TAIL_ROWS], w2_v[pl.ds(r0, W2_TAIL_ROWS), :],
                            preferred_element_type=f32)
    o_ref[...] = out.astype(o_ref.dtype)


@jax.jit
def pallas_sequential_preLN__sliding_block_cached__glu_gated_swiglu__decode_kernel(
    A_x: jax.Array,
    A_k_cache: jax.Array,
    A_v_cache: jax.Array,
    A_wq: jax.Array,
    A_wo: jax.Array,
    B_x: jax.Array,
    B_w1: jax.Array,
    B_w3: jax.Array,
    B_w2: jax.Array,
):
    B, Sq, D = A_x.shape
    _, hkv, sk, dh = A_k_cache.shape
    assert (B, Sq, hkv, dh) == (1, 1, HQ, DH)
    win = min(4096, max(256, sk // 4))
    ff = B_w1.shape[1]
    bf16, f32 = jnp.bfloat16, jnp.float32
    n_tail = (ff - W2_EARLY) // W2_TAIL_ROWS

    kt = jnp.swapaxes(A_k_cache, 2, 3).reshape(HQ, DH, sk)
    vt = jnp.swapaxes(A_v_cache, 2, 3).reshape(HQ, DH, sk)
    x2 = A_x.reshape(1, D)
    wo3 = A_wo.reshape(HQ, DH, D)

    any_spec = pl.BlockSpec(memory_space=pl.ANY)
    out = pl.pallas_call(
        functools.partial(_kernel, win=win, sk=sk),
        out_shape=jax.ShapeDtypeStruct((1, D), A_x.dtype),
        in_specs=[any_spec] * 8,
        out_specs=pl.BlockSpec(memory_space=pltpu.VMEM),
        scratch_shapes=[
            pltpu.VMEM((1, D), bf16),
            pltpu.VMEM((HQ // 2, D, 2 * DH), bf16),
            pltpu.VMEM((HQ, DH, D), bf16),
            pltpu.VMEM((D, ff), bf16),
            pltpu.VMEM((D, ff), bf16),
            pltpu.VMEM((ff, D), bf16),
            pltpu.VMEM((NSLOT, DH, CW), bf16),
            pltpu.VMEM((win // CW, CW), f32),
            pltpu.VMEM((win // CW, CW), f32),
            pltpu.VMEM((1, D), f32),
            pltpu.SemaphoreType.DMA((NSLOT * TPC,)),
            pltpu.SemaphoreType.DMA((3,)),
            pltpu.SemaphoreType.DMA((2,)),
            pltpu.SemaphoreType.DMA((4,)),
            pltpu.SemaphoreType.DMA((n_tail,)),
        ],
        compiler_params=pltpu.CompilerParams(
            vmem_limit_bytes=64 * 1024 * 1024,
            disable_bounds_checks=CHECKS_OFF,
            disable_semaphore_checks=CHECKS_OFF),
    )(x2, kt, vt, A_wq, wo3, B_w1, B_w3, B_w2)
    return out.reshape(B, Sq, D)
```

```python
import functools

import jax
import jax.numpy as jnp
import jax.experimental.pallas as pl
import jax.experimental.pallas.tpu as pltpu

HQ = 32
DH = 192
EPS = 1e-5
LANE = 128
TW = 128
TPC = 4
CW = TW * TPC
LOOK = 16
NSLOT = 8
BULK = 1
TRICKLE = 0
WQ_ROWS = 32
WO_COLS = (0,384,640)
W13_COLS = 512
W13_FRAC = (0.54, 0.94)
LATE0 = 100
W2_EARLY = 192
W2_SPLIT = 384
W2_MXU_ROWS = 128
W2_VPU_ROWS = 64
W2_VPU_CHUNKS = 2
W2_MERGE = 7
OPROJ_AT = 3
QPROJ_AT = 6
CHECKS_OFF = True
COMPUTE = True


def _layernorm(x):
    m = jnp.mean(x, axis=-1, keepdims=True)
    xc = x - m
    v = jnp.mean(xc * xc, axis=-1, keepdims=True)
    return xc * jax.lax.rsqrt(v + EPS)


def _merge(groups):
    items = []
    for g in groups:
        for k, it in enumerate(g):
            items.append(((k + 0.5) / len(g), it))
    items.sort(key=lambda t: t[0])
    return [it for _, it in items]


def _place(items, n):
    slots = [[] for _ in range(n)]
    for k, it in enumerate(items):
        slots[k * n // len(items)].append(it)
    return slots


def _tail_chunks(ff):
    n_vpu_rows = W2_VPU_ROWS * W2_VPU_CHUNKS
    chunks, r = [], W2_EARLY
    while r < ff - n_vpu_rows:
        nr = min(W2_MXU_ROWS - r % W2_MXU_ROWS, ff - n_vpu_rows - r)
        chunks.append((r, nr))
        r += nr
    n_mxu = len(chunks)
    for _ in range(W2_VPU_CHUNKS):
        chunks.append((r, W2_VPU_ROWS))
        r += W2_VPU_ROWS
    assert r == ff
    return chunks, n_mxu


def _kernel(x_hbm, kt_hbm, vt_hbm, wq_hbm, wo_hbm, w1_hbm, w3_hbm, w2_hbm,
            o_ref,
            x_v, wq_v, wo_v, w1_v, w3_v, w2_v, kvbuf, s_scr, p_scr, acc_s, ab_s,
            sem_kv, sem_q, sem_o, sem_w, sem_t, *, win, sk):
    f32, bf16 = jnp.float32, jnp.bfloat16
    col0 = sk - win
    d_model = x_v.shape[1]
    ff = w2_v.shape[0]
    nch = win // CW
    ntk = win // TW
    per_head = 2 * ntk
    npair = HQ // 2
    pw = 2 * DH
    nts = NSLOT * TPC
    w13r = d_model // npair
    tail, n_mxu = _tail_chunks(ff)
    assert per_head % nts == 0 and LOOK <= nts - TPC and len(tail) <= LOOK

    def aligned(v, m):
        return v if isinstance(v, int) else pl.multiple_of(v, m)

    def kv_copy(h, t):
        src = kt_hbm if t < ntk else vt_hbm
        c = t % ntk
        ts = t % nts
        return pltpu.make_async_copy(
            src.at[h, :, pl.ds(col0 + c * TW, TW)],
            kvbuf.at[ts // TPC, :, pl.ds((ts % TPC) * TW, TW)], sem_kv.at[ts])

    def wq_piece(blk, r0, nr, c0, nc):
        s = blk % 2 if isinstance(blk, int) else jax.lax.rem(blk, 2)
        return pltpu.make_async_copy(
            wq_hbm.at[pl.ds(r0, nr), pl.ds(aligned(blk * pw + c0, LANE), nc)],
            wq_v.at[blk, pl.ds(r0, nr), pl.ds(c0, nc)], sem_q.at[s])

    def wq_whole(blk):
        return wq_piece(blk, 0, d_model, 0, pw)

    def wo_piece(h, par, r0, nr, c0=0, nc=None):
        nc = d_model if nc is None else nc
        return pltpu.make_async_copy(
            wo_hbm.at[h, pl.ds(r0, nr), pl.ds(c0, nc)],
            wo_v.at[h, pl.ds(r0, nr), pl.ds(c0, nc)], sem_o.at[par])

    def w13_piece(which, pair, r, c0):
        src, dst = ((w1_hbm, w1_v), (w3_hbm, w3_v))[which]
        r0 = aligned(pair * w13r + r, 8)
        return pltpu.make_async_copy(
            src.at[pl.ds(r0, 8), pl.ds(c0, W13_COLS)],
            dst.at[pl.ds(r0, 8), pl.ds(c0, W13_COLS)], sem_w.at[1 + which])

    def w2_copy(r0, nr, c0, nc, sem):
        return pltpu.make_async_copy(
            w2_hbm.at[pl.ds(r0, nr), pl.ds(c0, nc)], w2_v.at[pl.ds(r0, nr), pl.ds(c0, nc)], sem)

    def w2_tail_copy(k):
        return w2_copy(tail[k][0], tail[k][1], 0, d_model, sem_t.at[k])

    x_copy = pltpu.make_async_copy(x_hbm, x_v, sem_w.at[0])

    def q_project(blk, xn):
        q = jnp.dot(xn, wq_v[blk], preferred_element_type=f32) * (DH ** -0.5)
        return q[:, :DH], q[:, DH:]

    wq_l = [("wq", r0, c0) for r0 in range(0, d_model, WQ_ROWS) for c0 in range(0, pw, LANE)]
    wo_l = [[("wo", par, r0, c0, c1 - c0) for r0 in range(0, DH, 8)
             for c0, c1 in zip(WO_COLS[:-1], WO_COLS[1:])] for par in range(2)]
    w13_l = [("w13", w, r, c0) for r in range(0, w13r, 8) for w in range(2)
             for c0 in range(0, ff, W13_COLS)]
    w2_l = [("w2", r0) + cs for r0 in range(0, W2_EARLY, 8)
            for cs in ((0, W2_SPLIT), (W2_SPLIT, d_model - W2_SPLIT))]
    def pair_up(normal, last):
        n = max(len(normal), len(last))
        na = {k * n // len(normal): it for k, it in enumerate(normal)} if normal else {}
        la = {k * n // len(last): it for k, it in enumerate(last)} if last else {}
        return [(na.get(k), la.get(k)) for k in range(n)]

    n_mid, n_late = LATE0 - per_head, 2 * per_head - LATE0
    nq_a, n2_a = len(wq_l) // 2, len(w2_l) // 2
    f_a, f_b = W13_FRAC
    n13_a, n13_b = int(len(w13_l) * f_a), int(len(w13_l) * f_b)
    both = lambda g: [(it, it) for it in g]
    sched = (
        _place(_merge([both(wo_l[0]), pair_up(wq_l[:nq_a], w2_l[:n2_a]),
                       both(w13_l[:n13_a])]), per_head)
        + _place(_merge([pair_up(wq_l[nq_a:], wo_l[1]), both(w13_l[n13_a:n13_b])]), n_mid)
        + _place(both(w13_l[n13_b:]) + pair_up(wo_l[1], w2_l[n2_a:]), n_late))
    flat = [it for slot in sched for it in slot]
    assert len(sched) == 2 * per_head
    assert DH % 8 == 0 and d_model % WQ_ROWS == 0 and d_model % (8 * npair) == 0
    assert ff % W13_COLS == 0 and W2_EARLY % 8 == 0
    assert sorted(n for n, _ in flat if n) == sorted(wq_l + wo_l[0] + wo_l[1] + w13_l)
    assert sorted(l for _, l in flat if l) == sorted(w2_l + wo_l[0] + wo_l[1] + w13_l)

    x_copy.start(priority=TRICKLE)
    wq_whole(0).start(priority=TRICKLE)

    def first_ticks(j, carry):
        for u in range(TPC):
            pltpu.make_async_copy(
                kt_hbm.at[0, :, pl.ds(pl.multiple_of(col0 + (j * TPC + u) * TW, LANE), TW)],
                kvbuf.at[j, :, pl.ds(u * TW, TW)], sem_kv.at[j * TPC + u]).start(priority=BULK)
        return carry

    assert LOOK % TPC == 0 and LOOK <= ntk
    jax.lax.fori_loop(0, LOOK // TPC, first_ticks, 0)
    x_copy.wait()
    x = x_v[...].astype(f32)
    xn = _layernorm(x).astype(bf16)
    acc_s[...] = jnp.zeros_like(acc_s)
    wq_whole(0).wait()
    q0 = q_project(0, xn)

    def pair_body(pair, carry):
        q_cur, o_prev = carry[:2], carry[2]
        q_next = q_cur
        not_last = pair + 1 < npair

        def piece(it):
            if it[0] == "wo":
                return wo_piece(2 * pair + it[1], it[1], it[2], 8, it[3], it[4])
            if it[0] == "w13":
                return w13_piece(it[1], pair, it[2], it[3])
            if it[0] == "wq":
                return wq_piece(pair + 1, it[1], WQ_ROWS, it[2], LANE)
            return w2_copy(it[1], 8, it[2], it[3], sem_w.at[3])

        def tick(par, t):
            h = 2 * pair + par
            kv_copy(h, t).wait()
            t2 = t + LOOK
            if t2 < per_head:
                kv_copy(h, t2).start(priority=BULK)
            elif par == 0:
                kv_copy(h + 1, t2 - per_head).start(priority=BULK)
            else:
                @pl.when(not_last)
                def _():
                    kv_copy(h + 1, t2 - per_head).start(priority=BULK)

                if t2 - per_head < len(tail):
                    @pl.when(jnp.logical_not(not_last))
                    def _():
                        w2_tail_copy(t2 - per_head).start(priority=BULK)
            for normal, last in sched[par * per_head + t]:
                if normal == last:
                    piece(normal).start(priority=TRICKLE)
                    continue

                if normal is not None:
                    @pl.when(not_last)
                    def _():
                        piece(normal).start(priority=TRICKLE)

                if last is not None:
                    @pl.when(jnp.logical_not(not_last))
                    def _():
                        piece(last).start(priority=TRICKLE)

        def out_project(h, par, o_h):
            wo_piece(h, par, 0, DH).wait()
            if COMPUTE:
                acc_s[...] += jnp.dot(o_h.astype(bf16), wo_v[h], preferred_element_type=f32)

        for par in range(2):
            h = 2 * pair + par
            q = q_cur[par].astype(bf16)
            for c in range(nch):
                for u in range(TPC):
                    tick(par, c * TPC + u)
                    if u == 0 and c == OPROJ_AT:
                        if par == 1:
                            out_project(h - 1, 0, o_prev)
                        else:
                            @pl.when(pair > 0)
                            def _():
                                out_project(h - 1, 1, o_prev)
                if COMPUTE:
                    s_scr[c:c + 1, :] = jnp.dot(q, kvbuf[c % NSLOT], preferred_element_type=f32)
            o = jnp.zeros((1, DH), f32)
            l = jnp.ones((1, 1), f32)
            for c in range(nch):
                for u in range(TPC):
                    tick(par, ntk + c * TPC + u)
                    if u == 0 and c == 0 and COMPUTE:
                        s = s_scr[...]
                        m = jnp.max(jnp.max(s, axis=1, keepdims=True), axis=0, keepdims=True)
                        p = jnp.exp(s - m)
                        l = jnp.sum(jnp.sum(p, axis=1, keepdims=True), axis=0, keepdims=True)
                        p_scr[...] = p
                    if u == 0 and c == QPROJ_AT and par == 1:
                        @pl.when(not_last)
                        def _():
                            wq_whole(pair + 1).wait()

                        if COMPUTE:
                            q_next = q_project(jnp.minimum(pair + 1, npair - 1), xn)
                if COMPUTE:
                    o = o + jax.lax.dot_general(p_scr[c:c + 1, :].astype(bf16),
                                                kvbuf[(nch + c) % NSLOT],
                                                (((1,), (1,)), ((), ())),
                                                preferred_element_type=f32)
            o_prev = o / l
        return (q_next[0], q_next[1], o_prev)

    _, _, o_last = jax.lax.fori_loop(
        0, npair, pair_body, (q0[0], q0[1], jnp.zeros((1, DH), f32)))

    wo_piece(HQ - 1, 1, 0, DH).wait()
    attn = acc_s[...] + jnp.dot(o_last.astype(bf16), wo_v[HQ - 1], preferred_element_type=f32)
    hres = x + attn
    hn = _layernorm(hres).astype(bf16)
    pltpu.make_async_copy(w1_hbm, w1_v, sem_w.at[1]).wait()
    pltpu.make_async_copy(w3_hbm, w3_v, sem_w.at[2]).wait()
    w2_copy(0, W2_EARLY, 0, d_model, sem_w.at[3]).wait()
    g = jnp.dot(hn, w1_v[...], preferred_element_type=f32)
    u = jnp.dot(hn, w3_v[...], preferred_element_type=f32)
    a = (g * jax.nn.sigmoid(g) * u).astype(bf16)
    nv = W2_VPU_ROWS * W2_VPU_CHUNKS
    a_end = jnp.broadcast_to(a[:, ff - nv:].astype(f32), (nv, nv))
    diag = (jax.lax.broadcasted_iota(jnp.int32, (nv, nv), 0)
            == jax.lax.broadcasted_iota(jnp.int32, (nv, nv), 1))
    a_col = jnp.sum(jnp.where(diag, a_end, 0.0), axis=1, keepdims=True)
    ab_s[...] = jnp.broadcast_to(a_col, ab_s.shape)
    for k in range(W2_MERGE):
        w2_tail_copy(k).wait()
    r1 = tail[W2_MERGE][0]
    out = hres + jnp.dot(a[:, :r1], w2_v[pl.ds(0, r1), :], preferred_element_type=f32)
    for k in range(W2_MERGE, n_mxu):
        r0, nr = tail[k]
        w2_tail_copy(k).wait()
        out = out + jnp.dot(a[:, r0:r0 + nr], w2_v[pl.ds(r0, nr), :],
                            preferred_element_type=f32)
    part = None
    for k in range(n_mxu, len(tail)):
        r0, nr = tail[k]
        w2_tail_copy(k).wait()
        for rg in range(0, nr, 8):
            ab = ab_s[pl.ds(r0 - (ff - nv) + rg, 8), :]
            term = (w2_v[pl.ds(r0 + rg, 8), :].astype(f32)
                    * jnp.concatenate([ab] * (d_model // LANE), axis=1))
            part = term if part is None else part + term
    out = out + jnp.sum(part, axis=0, keepdims=True)
    o_ref[...] = out.astype(o_ref.dtype)


@jax.jit
def pallas_sequential_preLN__sliding_block_cached__glu_gated_swiglu__decode_kernel(
    A_x: jax.Array,
    A_k_cache: jax.Array,
    A_v_cache: jax.Array,
    A_wq: jax.Array,
    A_wo: jax.Array,
    B_x: jax.Array,
    B_w1: jax.Array,
    B_w3: jax.Array,
    B_w2: jax.Array,
):
    B, Sq, D = A_x.shape
    _, hkv, sk, dh = A_k_cache.shape
    assert (B, Sq, hkv, dh) == (1, 1, HQ, DH)
    win = min(4096, max(256, sk // 4))
    ff = B_w1.shape[1]
    bf16, f32 = jnp.bfloat16, jnp.float32
    n_tail = len(_tail_chunks(ff)[0])

    kt = jnp.swapaxes(A_k_cache, 2, 3).reshape(HQ, DH, sk)
    vt = jnp.swapaxes(A_v_cache, 2, 3).reshape(HQ, DH, sk)
    x2 = A_x.reshape(1, D)
    wo3 = A_wo.reshape(HQ, DH, D)

    any_spec = pl.BlockSpec(memory_space=pl.ANY)
    out = pl.pallas_call(
        functools.partial(_kernel, win=win, sk=sk),
        out_shape=jax.ShapeDtypeStruct((1, D), A_x.dtype),
        in_specs=[any_spec] * 8,
        out_specs=pl.BlockSpec(memory_space=pltpu.VMEM),
        scratch_shapes=[
            pltpu.VMEM((1, D), bf16),
            pltpu.VMEM((HQ // 2, D, 2 * DH), bf16),
            pltpu.VMEM((HQ, DH, D), bf16),
            pltpu.VMEM((D, ff), bf16),
            pltpu.VMEM((D, ff), bf16),
            pltpu.VMEM((ff, D), bf16),
            pltpu.VMEM((NSLOT, DH, CW), bf16),
            pltpu.VMEM((win // CW, CW), f32),
            pltpu.VMEM((win // CW, CW), f32),
            pltpu.VMEM((1, D), f32),
            pltpu.VMEM((W2_VPU_ROWS * W2_VPU_CHUNKS, LANE), f32),
            pltpu.SemaphoreType.DMA((NSLOT * TPC,)),
            pltpu.SemaphoreType.DMA((2,)),
            pltpu.SemaphoreType.DMA((2,)),
            pltpu.SemaphoreType.DMA((4,)),
            pltpu.SemaphoreType.DMA((n_tail,)),
        ],
        compiler_params=pltpu.CompilerParams(
            vmem_limit_bytes=64 * 1024 * 1024,
            disable_bounds_checks=CHECKS_OFF,
            disable_semaphore_checks=CHECKS_OFF),
    )(x2, kt, vt, A_wq, wo3, B_w1, B_w3, B_w2)
    return out.reshape(B, Sq, D)
```

```python
import functools

import jax
import jax.numpy as jnp
import jax.experimental.pallas as pl
import jax.experimental.pallas.tpu as pltpu

HQ = 32
DH = 192
EPS = 1e-5
LANE = 128
TW = 128
TPC = 4
CW = TW * TPC
LOOK = 16
NSLOT = 8
BULK = 1
TRICKLE = 0
WQ_ROWS = 32
WO_COLS = (0, 128, 256, 384, 512, 640)
W13_COLS = 512
W13_FRAC = (0.54, 0.94)
LATE0 = 92
W2_EARLY = 128
W2_SPLIT = 384
W2_MXU_ROWS = 128
W2_VPU_ROWS = 64
W2_VPU_CHUNKS = 2
W2_MERGE = 7
OPROJ_AT = 3
QPROJ_AT = 4


def _layernorm(x):
    m = jnp.mean(x, axis=-1, keepdims=True)
    xc = x - m
    v = jnp.mean(xc * xc, axis=-1, keepdims=True)
    return xc * jax.lax.rsqrt(v + EPS)


def _merge(groups):
    items = []
    for g in groups:
        for k, it in enumerate(g):
            items.append(((k + 0.5) / len(g), it))
    items.sort(key=lambda t: t[0])
    return [it for _, it in items]


def _place(items, n):
    slots = [[] for _ in range(n)]
    for k, it in enumerate(items):
        slots[k * n // len(items)].append(it)
    return slots


def _pair_up(normal, last):
    n = max(len(normal), len(last))
    na = {k * n // len(normal): it for k, it in enumerate(normal)} if normal else {}
    la = {k * n // len(last): it for k, it in enumerate(last)} if last else {}
    return [(na.get(k), la.get(k)) for k in range(n)]


def _tail_chunks(ff):
    n_vpu_rows = W2_VPU_ROWS * W2_VPU_CHUNKS
    chunks, r = [], W2_EARLY
    while r < ff - n_vpu_rows:
        nr = min(W2_MXU_ROWS - r % W2_MXU_ROWS, ff - n_vpu_rows - r)
        chunks.append((r, nr))
        r += nr
    n_mxu = len(chunks)
    for _ in range(W2_VPU_CHUNKS):
        chunks.append((r, W2_VPU_ROWS))
        r += W2_VPU_ROWS
    assert r == ff
    return chunks, n_mxu


def _trickle_schedule(d_model, ff, per_head, npair):
    pw, w13r = 2 * DH, d_model // npair
    wq_l = [("wq", r0, c0) for r0 in range(0, d_model, WQ_ROWS) for c0 in range(0, pw, LANE)]
    wo_l = [[("wo", par, r0, c0, c1 - c0) for r0 in range(0, DH, 8)
             for c0, c1 in zip(WO_COLS[:-1], WO_COLS[1:])] for par in range(2)]
    w13_l = [("w13", w, r, c0) for r in range(0, w13r, 8) for w in range(2)
             for c0 in range(0, ff, W13_COLS)]
    w2_l = [("w2", r0) + cs for r0 in range(0, W2_EARLY, 8)
            for cs in ((0, W2_SPLIT), (W2_SPLIT, d_model - W2_SPLIT))]
    n_mid, n_late = LATE0 - per_head, 2 * per_head - LATE0
    nq_a, n2_a = len(wq_l) // 2, len(w2_l) // 2
    n13_a, n13_b = (int(len(w13_l) * f) for f in W13_FRAC)

    def both(g):
        return [(it, it) for it in g]

    sched = (
        _place(_merge([both(wo_l[0]), _pair_up(wq_l[:nq_a], w2_l[:n2_a]),
                       both(w13_l[:n13_a])]), per_head)
        + _place(_merge([_pair_up(wq_l[nq_a:], wo_l[1]), both(w13_l[n13_a:n13_b])]), n_mid)
        + _place(both(w13_l[n13_b:]) + _pair_up(wo_l[1], w2_l[n2_a:]), n_late))
    flat = [it for slot in sched for it in slot]
    assert len(sched) == 2 * per_head
    assert DH % 8 == 0 and d_model % WQ_ROWS == 0 and d_model % (8 * npair) == 0
    assert ff % W13_COLS == 0 and W2_EARLY % 8 == 0
    assert WO_COLS[0] == 0 and WO_COLS[-1] == d_model
    assert sorted(n for n, _ in flat if n) == sorted(wq_l + wo_l[0] + wo_l[1] + w13_l)
    assert sorted(l for _, l in flat if l) == sorted(w2_l + wo_l[0] + wo_l[1] + w13_l)
    return sched


def _kernel(x_hbm, kt_hbm, vt_hbm, wq_hbm, wo_hbm, w1_hbm, w3_hbm, w2_hbm,
            o_ref,
            x_v, wq_v, wo_v, w1_v, w3_v, w2_v, kvbuf, s_scr, p_scr, acc_s, ab_s,
            sem_kv, sem_q, sem_o, sem_w, sem_t, *, win, sk):
    f32, bf16 = jnp.float32, jnp.bfloat16
    col0 = sk - win
    d_model = x_v.shape[1]
    ff = w2_v.shape[0]
    nch = win // CW
    ntk = win // TW
    per_head = 2 * ntk
    npair = HQ // 2
    pw = 2 * DH
    nts = NSLOT * TPC
    w13r = d_model // npair
    tail, n_mxu = _tail_chunks(ff)
    sched = _trickle_schedule(d_model, ff, per_head, npair)
    assert per_head % nts == 0 and LOOK <= nts - TPC and len(tail) <= LOOK
    assert LOOK % TPC == 0 and LOOK <= ntk and col0 % LANE == 0
    assert per_head + ntk + QPROJ_AT * TPC >= LATE0 and W2_MERGE < n_mxu

    def aligned(v, m):
        return v if isinstance(v, int) else pl.multiple_of(v, m)

    def kv_copy(h, t):
        src = kt_hbm if t < ntk else vt_hbm
        c = t % ntk
        ts = t % nts
        return pltpu.make_async_copy(
            src.at[h, :, pl.ds(col0 + c * TW, TW)],
            kvbuf.at[ts // TPC, :, pl.ds((ts % TPC) * TW, TW)], sem_kv.at[ts])

    def wq_piece(blk, r0, nr, c0, nc):
        s = blk % 2 if isinstance(blk, int) else jax.lax.rem(blk, 2)
        return pltpu.make_async_copy(
            wq_hbm.at[pl.ds(r0, nr), pl.ds(aligned(blk * pw + c0, LANE), nc)],
            wq_v.at[blk, pl.ds(r0, nr), pl.ds(c0, nc)], sem_q.at[s])

    def wq_whole(blk):
        return wq_piece(blk, 0, d_model, 0, pw)

    def wo_piece(h, par, r0, nr, c0, nc):
        return pltpu.make_async_copy(
            wo_hbm.at[h, pl.ds(r0, nr), pl.ds(c0, nc)],
            wo_v.at[h, pl.ds(r0, nr), pl.ds(c0, nc)], sem_o.at[par])

    def wo_whole(h, par):
        return wo_piece(h, par, 0, DH, 0, d_model)

    def w13_piece(which, pair, r, c0):
        src, dst = ((w1_hbm, w1_v), (w3_hbm, w3_v))[which]
        r0 = aligned(pair * w13r + r, 8)
        return pltpu.make_async_copy(
            src.at[pl.ds(r0, 8), pl.ds(c0, W13_COLS)],
            dst.at[pl.ds(r0, 8), pl.ds(c0, W13_COLS)], sem_w.at[1 + which])

    def w2_copy(r0, nr, c0, nc, sem):
        return pltpu.make_async_copy(
            w2_hbm.at[pl.ds(r0, nr), pl.ds(c0, nc)], w2_v.at[pl.ds(r0, nr), pl.ds(c0, nc)], sem)

    def w2_tail_copy(k):
        return w2_copy(tail[k][0], tail[k][1], 0, d_model, sem_t.at[k])

    x_copy = pltpu.make_async_copy(x_hbm, x_v, sem_w.at[0])

    def q_project(blk, xn):
        q = jnp.dot(xn, wq_v[blk], preferred_element_type=f32) * (DH ** -0.5)
        return q[:, :DH], q[:, DH:]

    x_copy.start(priority=TRICKLE)
    wq_whole(0).start(priority=TRICKLE)

    def first_ticks(j, carry):
        for u in range(TPC):
            pltpu.make_async_copy(
                kt_hbm.at[0, :, pl.ds(pl.multiple_of(col0 + (j * TPC + u) * TW, LANE), TW)],
                kvbuf.at[j, :, pl.ds(u * TW, TW)], sem_kv.at[j * TPC + u]).start(priority=BULK)
        return carry

    jax.lax.fori_loop(0, LOOK // TPC, first_ticks, 0)
    x_copy.wait()
    x = x_v[...].astype(f32)
    xn = _layernorm(x).astype(bf16)
    acc_s[...] = jnp.zeros_like(acc_s)
    wq_whole(0).wait()
    q0 = q_project(0, xn)

    def pair_body(pair, carry):
        q_cur, o_prev = carry[:2], carry[2]
        q_next = q_cur
        not_last = pair + 1 < npair
        is_last = pair + 1 == npair

        def piece(it):
            if it[0] == "wo":
                return wo_piece(2 * pair + it[1], it[1], it[2], 8, it[3], it[4])
            if it[0] == "w13":
                return w13_piece(it[1], pair, it[2], it[3])
            if it[0] == "wq":
                return wq_piece(pair + 1, it[1], WQ_ROWS, it[2], LANE)
            return w2_copy(it[1], 8, it[2], it[3], sem_w.at[3])

        def tick(par, t):
            h = 2 * pair + par
            kv_copy(h, t).wait()
            t2 = t + LOOK
            if t2 < per_head:
                kv_copy(h, t2).start(priority=BULK)
            elif par == 0:
                kv_copy(h + 1, t2 - per_head).start(priority=BULK)
            else:
                @pl.when(not_last)
                def _():
                    kv_copy(h + 1, t2 - per_head).start(priority=BULK)

                if t2 - per_head < len(tail):
                    @pl.when(is_last)
                    def _():
                        w2_tail_copy(t2 - per_head).start(priority=BULK)
            for normal, last in sched[par * per_head + t]:
                if normal == last:
                    piece(normal).start(priority=TRICKLE)
                    continue
                if normal is not None:
                    @pl.when(not_last)
                    def _():
                        piece(normal).start(priority=TRICKLE)
                if last is not None:
                    @pl.when(is_last)
                    def _():
                        piece(last).start(priority=TRICKLE)

        def out_project(h, par, o_h):
            wo_whole(h, par).wait()
            acc_s[...] += jnp.dot(o_h.astype(bf16), wo_v[h], preferred_element_type=f32)

        for par in range(2):
            h = 2 * pair + par
            q = q_cur[par].astype(bf16)
            for c in range(nch):
                for u in range(TPC):
                    tick(par, c * TPC + u)
                    if u == 0 and c == OPROJ_AT:
                        if par == 1:
                            out_project(h - 1, 0, o_prev)
                        else:
                            @pl.when(pair > 0)
                            def _():
                                out_project(h - 1, 1, o_prev)
                s_scr[c:c + 1, :] = jnp.dot(q, kvbuf[c % NSLOT], preferred_element_type=f32)
            o = jnp.zeros((1, DH), f32)
            for c in range(nch):
                for u in range(TPC):
                    tick(par, ntk + c * TPC + u)
                    if u == 0 and c == 0:
                        s = s_scr[...]
                        m = jnp.max(jnp.max(s, axis=1, keepdims=True), axis=0, keepdims=True)
                        p = jnp.exp(s - m)
                        l = jnp.sum(jnp.sum(p, axis=1, keepdims=True), axis=0, keepdims=True)
                        p_scr[...] = p
                    if u == 0 and c == QPROJ_AT and par == 1:
                        @pl.when(not_last)
                        def _():
                            wq_whole(pair + 1).wait()

                        q_next = q_project(jnp.minimum(pair + 1, npair - 1), xn)
                o = o + jax.lax.dot_general(p_scr[c:c + 1, :].astype(bf16),
                                            kvbuf[(nch + c) % NSLOT],
                                            (((1,), (1,)), ((), ())),
                                            preferred_element_type=f32)
            o_prev = o / l
        return (q_next[0], q_next[1], o_prev)

    _, _, o_last = jax.lax.fori_loop(
        0, npair, pair_body, (q0[0], q0[1], jnp.zeros((1, DH), f32)))

    wo_whole(HQ - 1, 1).wait()
    attn = acc_s[...] + jnp.dot(o_last.astype(bf16), wo_v[HQ - 1], preferred_element_type=f32)
    hres = x + attn
    hn = _layernorm(hres).astype(bf16)
    pltpu.make_async_copy(w1_hbm, w1_v, sem_w.at[1]).wait()
    pltpu.make_async_copy(w3_hbm, w3_v, sem_w.at[2]).wait()
    w2_copy(0, W2_EARLY, 0, d_model, sem_w.at[3]).wait()
    g = jnp.dot(hn, w1_v[...], preferred_element_type=f32)
    u = jnp.dot(hn, w3_v[...], preferred_element_type=f32)
    a = (g * jax.nn.sigmoid(g) * u).astype(bf16)
    for k in range(W2_MERGE):
        w2_tail_copy(k).wait()
    nv = W2_VPU_ROWS * W2_VPU_CHUNKS
    a_end = jnp.broadcast_to(a[:, ff - nv:].astype(f32), (nv, nv))
    diag = (jax.lax.broadcasted_iota(jnp.int32, (nv, nv), 0)
            == jax.lax.broadcasted_iota(jnp.int32, (nv, nv), 1))
    a_col = jnp.sum(jnp.where(diag, a_end, 0.0), axis=1, keepdims=True)
    ab_s[...] = jnp.broadcast_to(a_col, ab_s.shape)
    r1 = tail[W2_MERGE][0]
    out = hres + jnp.dot(a[:, :r1], w2_v[pl.ds(0, r1), :], preferred_element_type=f32)
    for k in range(W2_MERGE, n_mxu):
        r0, nr = tail[k]
        w2_tail_copy(k).wait()
        out = out + jnp.dot(a[:, r0:r0 + nr], w2_v[pl.ds(r0, nr), :],
                            preferred_element_type=f32)
    part = None
    for k in range(n_mxu, len(tail)):
        r0, nr = tail[k]
        w2_tail_copy(k).wait()
        for rg in range(0, nr, 8):
            ab = ab_s[pl.ds(r0 - (ff - nv) + rg, 8), :]
            term = (w2_v[pl.ds(r0 + rg, 8), :].astype(f32)
                    * jnp.concatenate([ab] * (d_model // LANE), axis=1))
            part = term if part is None else part + term
    out = out + jnp.sum(part, axis=0, keepdims=True)
    o_ref[...] = out.astype(o_ref.dtype)


@jax.jit
def pallas_sequential_preLN__sliding_block_cached__glu_gated_swiglu__decode_kernel(
    A_x: jax.Array,
    A_k_cache: jax.Array,
    A_v_cache: jax.Array,
    A_wq: jax.Array,
    A_wo: jax.Array,
    B_x: jax.Array,
    B_w1: jax.Array,
    B_w3: jax.Array,
    B_w2: jax.Array,
):
    B, Sq, D = A_x.shape
    _, hkv, sk, dh = A_k_cache.shape
    assert (B, Sq, hkv, dh) == (1, 1, HQ, DH)
    win = min(4096, max(256, sk // 4))
    ff = B_w1.shape[1]
    bf16, f32 = jnp.bfloat16, jnp.float32
    n_tail = len(_tail_chunks(ff)[0])

    kt = jnp.swapaxes(A_k_cache, 2, 3).reshape(HQ, DH, sk)
    vt = jnp.swapaxes(A_v_cache, 2, 3).reshape(HQ, DH, sk)
    x2 = A_x.reshape(1, D)
    wo3 = A_wo.reshape(HQ, DH, D)

    any_spec = pl.BlockSpec(memory_space=pl.ANY)
    out = pl.pallas_call(
        functools.partial(_kernel, win=win, sk=sk),
        out_shape=jax.ShapeDtypeStruct((1, D), A_x.dtype),
        in_specs=[any_spec] * 8,
        out_specs=pl.BlockSpec(memory_space=pltpu.VMEM),
        scratch_shapes=[
            pltpu.VMEM((1, D), bf16),
            pltpu.VMEM((HQ // 2, D, 2 * DH), bf16),
            pltpu.VMEM((HQ, DH, D), bf16),
            pltpu.VMEM((D, ff), bf16),
            pltpu.VMEM((D, ff), bf16),
            pltpu.VMEM((ff, D), bf16),
            pltpu.VMEM((NSLOT, DH, CW), bf16),
            pltpu.VMEM((win // CW, CW), f32),
            pltpu.VMEM((win // CW, CW), f32),
            pltpu.VMEM((1, D), f32),
            pltpu.VMEM((W2_VPU_ROWS * W2_VPU_CHUNKS, LANE), f32),
            pltpu.SemaphoreType.DMA((NSLOT * TPC,)),
            pltpu.SemaphoreType.DMA((2,)),
            pltpu.SemaphoreType.DMA((2,)),
            pltpu.SemaphoreType.DMA((4,)),
            pltpu.SemaphoreType.DMA((n_tail,)),
        ],
        compiler_params=pltpu.CompilerParams(
            vmem_limit_bytes=64 * 1024 * 1024,
            disable_bounds_checks=True,
            disable_semaphore_checks=True),
    )(x2, kt, vt, A_wq, wo3, B_w1, B_w3, B_w2)
    return out.reshape(B, Sq, D)
```

```python
import functools

import jax
import jax.numpy as jnp
import jax.experimental.pallas as pl
import jax.experimental.pallas.tpu as pltpu

HQ = 32
DH = 192
EPS = 1e-5
LANE = 128
TW = 128
TPC = 4
CW = TW * TPC
LOOK = 20
NSLOT = 8
BULK = 1
TRICKLE = 0
WO_COLS = (0, 384, 640)
W13_COLS = 384
W13_A = 0.56
LATE0 = 92
W2_EARLY = 128
W2_SPLIT = 384
W2_MXU_ROWS = 128
W2_VPU_ROWS = 64
W2_VPU_CHUNKS = 2
W2_MERGE = 7
OPROJ_AT = 3
QPROJ_AT = 4


def _layernorm(x):
    m = jnp.mean(x, axis=-1, keepdims=True)
    xc = x - m
    v = jnp.mean(xc * xc, axis=-1, keepdims=True)
    return xc * jax.lax.rsqrt(v + EPS)


def _merge(groups):
    items = []
    for g in groups:
        for k, it in enumerate(g):
            items.append(((k + 0.5) / len(g), it))
    items.sort(key=lambda t: t[0])
    return [it for _, it in items]


def _place(items, n):
    slots = [[] for _ in range(n)]
    for k, it in enumerate(items):
        slots[k * n // len(items)].append(it)
    return slots


def _pair_up(normal, last):
    n = max(len(normal), len(last))
    na = {k * n // len(normal): it for k, it in enumerate(normal)} if normal else {}
    la = {k * n // len(last): it for k, it in enumerate(last)} if last else {}
    return [(na.get(k), la.get(k)) for k in range(n)]


def _tail_chunks(ff):
    n_vpu_rows = W2_VPU_ROWS * W2_VPU_CHUNKS
    chunks, r = [], W2_EARLY
    while r < ff - n_vpu_rows:
        nr = min(W2_MXU_ROWS - r % W2_MXU_ROWS, ff - n_vpu_rows - r)
        chunks.append((r, nr))
        r += nr
    n_mxu = len(chunks)
    for _ in range(W2_VPU_CHUNKS):
        chunks.append((r, W2_VPU_ROWS))
        r += W2_VPU_ROWS
    assert r == ff
    return chunks, n_mxu


def _trickle_schedule(phase, d_model, ff, per_head, npair):
    wo_l = [[("wo", par, r0, c0, c1 - c0) for r0 in range(0, DH, 8)
             for c0, c1 in zip(WO_COLS[:-1], WO_COLS[1:])] for par in range(2)]

    def both(g):
        return [(it, it) for it in g]

    assert DH % 8 == 0 and WO_COLS[0] == 0 and WO_COLS[-1] == d_model
    if phase == 0:
        wq_l = [[("wq", par, k) for k in range(d_model // 8)] for par in range(2)]
        sched = sum((_place(_merge([both(wo_l[par]), both(wq_l[par])]), per_head)
                     for par in range(2)), [])
        want_n = want_l = wq_l[0] + wq_l[1] + wo_l[0] + wo_l[1]
    else:
        w13r = d_model // (npair // 2)
        w13_l = [("w13", w, r, c0) for r in range(0, w13r, 8) for w in range(2)
                 for c0 in range(0, ff, W13_COLS)]
        w2_l = [("w2", r0) + cs for r0 in range(0, W2_EARLY, 8)
                for cs in ((0, W2_SPLIT), (W2_SPLIT, d_model - W2_SPLIT))]
        n_mid, n_late = LATE0 - per_head, 2 * per_head - LATE0
        n13_a = int(len(w13_l) * W13_A)
        sched = (
            _place(_merge([both(wo_l[0]), both(w13_l[:n13_a])]), per_head)
            + _place(_merge([_pair_up([], wo_l[1]), both(w13_l[n13_a:])]), n_mid)
            + _place(_pair_up(wo_l[1], w2_l), n_late))
        assert ff % W13_COLS == 0 and W2_EARLY % 8 == 0 and w13r % 8 == 0
        want_n = wo_l[0] + wo_l[1] + w13_l
        want_l = want_n + w2_l
    flat = [it for slot in sched for it in slot]
    assert len(sched) == 2 * per_head
    assert sorted(n for n, _ in flat if n) == sorted(want_n)
    assert sorted(l for _, l in flat if l) == sorted(want_l)
    return sched


def _kernel(x_hbm, kt_hbm, vt_hbm, wq_hbm, wo_hbm, w1_hbm, w3_hbm, w2_hbm,
            o_ref,
            x_v, wq_v, wo_v, w1_v, w3_v, w2_v, kvbuf, s_scr, p_scr, acc_s, ab_s,
            sem_kv, sem_q, sem_o, sem_w, sem_t, *, win, sk):
    f32, bf16 = jnp.float32, jnp.bfloat16
    col0 = sk - win
    d_model = x_v.shape[1]
    ff = w2_v.shape[0]
    nch = win // CW
    ntk = win // TW
    per_head = 2 * ntk
    npair = HQ // 2
    pw = 2 * DH
    nts = NSLOT * TPC
    w13r = d_model // (npair // 2)
    nrg = d_model // 8
    nlev = npair.bit_length() - 1
    tail, n_mxu = _tail_chunks(ff)
    scheds = [_trickle_schedule(ph, d_model, ff, per_head, npair) for ph in range(2)]
    assert npair == 1 << nlev and nrg % (npair // 2) == 0
    assert per_head % nts == 0 and LOOK <= nts - TPC and len(tail) <= LOOK
    assert LOOK % TPC == 0 and LOOK <= ntk and col0 % LANE == 0
    assert per_head + ntk + QPROJ_AT * TPC >= LATE0 and W2_MERGE < n_mxu

    def aligned(v, m):
        return v if isinstance(v, int) else pl.multiple_of(v, m)

    def kv_copy(h, t):
        src = kt_hbm if t < ntk else vt_hbm
        c = t % ntk
        ts = t % nts
        return pltpu.make_async_copy(
            src.at[h, :, pl.ds(col0 + c * TW, TW)],
            kvbuf.at[ts // TPC, :, pl.ds((ts % TPC) * TW, TW)], sem_kv.at[ts])

    def wq_copy(blk, r0, nr, sem):
        return pltpu.make_async_copy(
            wq_hbm.at[pl.ds(r0, nr), pl.ds(aligned(blk * pw, LANE), pw)],
            wq_v.at[blk, pl.ds(r0, nr), :], sem)

    def wq_level_wait(lev):
        blocks = wq_v.at[pl.ds(1 << lev, 1 << lev)]
        pltpu.make_async_copy(blocks, blocks, sem_q.at[lev]).wait()

    def wo_piece(h, par, r0, nr, c0, nc):
        return pltpu.make_async_copy(
            wo_hbm.at[h, pl.ds(r0, nr), pl.ds(c0, nc)],
            wo_v.at[h, pl.ds(r0, nr), pl.ds(c0, nc)], sem_o.at[par])

    def wo_whole(h, par):
        return wo_piece(h, par, 0, DH, 0, d_model)

    def w13_piece(which, pair, r, c0):
        src, dst = ((w1_hbm, w1_v), (w3_hbm, w3_v))[which]
        r0 = aligned((pair - npair // 2) * w13r + r, 8)
        return pltpu.make_async_copy(
            src.at[pl.ds(r0, 8), pl.ds(c0, W13_COLS)],
            dst.at[pl.ds(r0, 8), pl.ds(c0, W13_COLS)], sem_w.at[1 + which])

    def w2_copy(r0, nr, c0, nc, sem):
        return pltpu.make_async_copy(
            w2_hbm.at[pl.ds(r0, nr), pl.ds(c0, nc)], w2_v.at[pl.ds(r0, nr), pl.ds(c0, nc)], sem)

    def w2_tail_copy(k):
        return w2_copy(tail[k][0], tail[k][1], 0, d_model, sem_t.at[k])

    x_copy = pltpu.make_async_copy(x_hbm, x_v, sem_w.at[0])

    def q_project(blk, xn):
        q = jnp.dot(xn, wq_v[blk], preferred_element_type=f32) * (DH ** -0.5)
        return q[:, :DH], q[:, DH:]

    x_copy.start(priority=TRICKLE)
    wq0_copy = wq_copy(0, 0, d_model, sem_w.at[4])
    wq0_copy.start(priority=TRICKLE)

    def first_ticks(j, carry):
        for u in range(TPC):
            pltpu.make_async_copy(
                kt_hbm.at[0, :, pl.ds(pl.multiple_of(col0 + (j * TPC + u) * TW, LANE), TW)],
                kvbuf.at[j, :, pl.ds(u * TW, TW)], sem_kv.at[j * TPC + u]).start(priority=BULK)
        return carry

    jax.lax.fori_loop(0, LOOK // TPC, first_ticks, 0)
    x_copy.wait()
    x = x_v[...].astype(f32)
    xn = _layernorm(x).astype(bf16)
    acc_s[...] = jnp.zeros_like(acc_s)
    wq0_copy.wait()
    q0 = q_project(0, xn)

    def pair_body(phase, pair, carry):
        q_cur, o_prev = carry[:2], carry[2]
        q_next = q_cur
        sched = scheds[phase]
        not_last = pair + 1 < npair
        is_last = pair + 1 == npair
        if phase == 0:
            levels = []
            for par in range(2):
                j1 = 2 * pair + par + 1
                lev = sum((j1 >= (2 << i)).astype(jnp.int32) for i in range(nlev - 1))
                nb = jax.lax.shift_left(jnp.int32(1), lev)
                rg0 = jax.lax.shift_right_logical((j1 - nb) * nrg, lev)
                levels.append((lev, nb, rg0))

        def piece(it):
            if it[0] == "wo":
                return wo_piece(2 * pair + it[1], it[1], it[2], 8, it[3], it[4])
            if it[0] == "w13":
                return w13_piece(it[1], pair, it[2], it[3])
            if it[0] == "wq":
                lev, nb, rg0 = levels[it[1]]
                k = jnp.int32(it[2])
                rg = rg0 + jax.lax.shift_right_logical(k, lev)
                return wq_copy(nb + (k & (nb - 1)), pl.multiple_of(rg * 8, 8), 8, sem_q.at[lev])
            return w2_copy(it[1], 8, it[2], it[3], sem_w.at[3])

        def tick(par, t):
            h = 2 * pair + par
            kv_copy(h, t).wait()
            t2 = t + LOOK
            if t2 < per_head:
                kv_copy(h, t2).start(priority=BULK)
            elif par == 0 or phase == 0:
                kv_copy(h + 1, t2 - per_head).start(priority=BULK)
            else:
                @pl.when(not_last)
                def _():
                    kv_copy(h + 1, t2 - per_head).start(priority=BULK)

                if t2 - per_head < len(tail):
                    @pl.when(is_last)
                    def _():
                        w2_tail_copy(t2 - per_head).start(priority=BULK)
            for normal, last in sched[par * per_head + t]:
                if normal is not None and normal[:2] == ("wq", 1):
                    @pl.when(pair + 1 < npair // 2)
                    def _():
                        piece(normal).start(priority=TRICKLE)
                    continue
                if normal == last:
                    piece(normal).start(priority=TRICKLE)
                    continue
                if normal is not None:
                    @pl.when(not_last)
                    def _():
                        piece(normal).start(priority=TRICKLE)
                if last is not None:
                    @pl.when(is_last)
                    def _():
                        piece(last).start(priority=TRICKLE)

        def out_project(h, par, o_h):
            wo_whole(h, par).wait()
            acc_s[...] += jnp.dot(o_h.astype(bf16), wo_v[h], preferred_element_type=f32)

        for par in range(2):
            h = 2 * pair + par
            q = q_cur[par].astype(bf16)
            for c in range(nch):
                for u in range(TPC):
                    tick(par, c * TPC + u)
                    if u == 0 and c == OPROJ_AT:
                        if par == 1 or phase == 1:
                            out_project(h - 1, 1 - par, o_prev)
                        else:
                            @pl.when(pair > 0)
                            def _():
                                out_project(h - 1, 1, o_prev)
                s_scr[c:c + 1, :] = jnp.dot(q, kvbuf[c % NSLOT], preferred_element_type=f32)
            o = jnp.zeros((1, DH), f32)
            for c in range(nch):
                for u in range(TPC):
                    tick(par, ntk + c * TPC + u)
                    if u == 0 and c == 0:
                        s = s_scr[...]
                        m = jnp.max(jnp.max(s, axis=1, keepdims=True), axis=0, keepdims=True)
                        p = jnp.exp(s - m)
                        l = jnp.sum(jnp.sum(p, axis=1, keepdims=True), axis=0, keepdims=True)
                        p_scr[...] = p
                    if u == 0 and c == QPROJ_AT and par == 1:
                        if phase == 0:
                            for lev in range(nlev):
                                @pl.when(pair + 1 == (1 << lev))
                                def _():
                                    wq_level_wait(lev)

                        q_next = q_project(jnp.minimum(pair + 1, npair - 1), xn)
                o = o + jax.lax.dot_general(p_scr[c:c + 1, :].astype(bf16),
                                            kvbuf[(nch + c) % NSLOT],
                                            (((1,), (1,)), ((), ())),
                                            preferred_element_type=f32)
            o_prev = o / l
        return (q_next[0], q_next[1], o_prev)

    carry = (q0[0], q0[1], jnp.zeros((1, DH), f32))
    carry = jax.lax.fori_loop(0, npair // 2, functools.partial(pair_body, 0), carry)
    carry = jax.lax.fori_loop(npair // 2, npair, functools.partial(pair_body, 1), carry)
    o_last = carry[2]

    wo_whole(HQ - 1, 1).wait()
    attn = acc_s[...] + jnp.dot(o_last.astype(bf16), wo_v[HQ - 1], preferred_element_type=f32)
    hres = x + attn
    hn = _layernorm(hres).astype(bf16)
    pltpu.make_async_copy(w1_hbm, w1_v, sem_w.at[1]).wait()
    pltpu.make_async_copy(w3_hbm, w3_v, sem_w.at[2]).wait()
    w2_copy(0, W2_EARLY, 0, d_model, sem_w.at[3]).wait()
    g = jnp.dot(hn, w1_v[...], preferred_element_type=f32)
    u = jnp.dot(hn, w3_v[...], preferred_element_type=f32)
    a = (g * jax.nn.sigmoid(g) * u).astype(bf16)
    for k in range(W2_MERGE):
        w2_tail_copy(k).wait()
    nv = W2_VPU_ROWS * W2_VPU_CHUNKS
    a_end = jnp.broadcast_to(a[:, ff - nv:].astype(f32), (nv, nv))
    diag = (jax.lax.broadcasted_iota(jnp.int32, (nv, nv), 0)
            == jax.lax.broadcasted_iota(jnp.int32, (nv, nv), 1))
    a_col = jnp.sum(jnp.where(diag, a_end, 0.0), axis=1, keepdims=True)
    ab_s[...] = jnp.broadcast_to(a_col, ab_s.shape)
    r1 = tail[W2_MERGE][0]
    out = hres + jnp.dot(a[:, :r1], w2_v[pl.ds(0, r1), :], preferred_element_type=f32)
    for k in range(W2_MERGE, n_mxu):
        r0, nr = tail[k]
        w2_tail_copy(k).wait()
        out = out + jnp.dot(a[:, r0:r0 + nr], w2_v[pl.ds(r0, nr), :],
                            preferred_element_type=f32)
    part = None
    for k in range(n_mxu, len(tail)):
        r0, nr = tail[k]
        w2_tail_copy(k).wait()
        for rg in range(0, nr, 8):
            ab = ab_s[pl.ds(r0 - (ff - nv) + rg, 8), :]
            term = (w2_v[pl.ds(r0 + rg, 8), :].astype(f32)
                    * jnp.concatenate([ab] * (d_model // LANE), axis=1))
            part = term if part is None else part + term
    out = out + jnp.sum(part, axis=0, keepdims=True)
    o_ref[...] = out.astype(o_ref.dtype)


@jax.jit
def pallas_sequential_preLN__sliding_block_cached__glu_gated_swiglu__decode_kernel(
    A_x: jax.Array,
    A_k_cache: jax.Array,
    A_v_cache: jax.Array,
    A_wq: jax.Array,
    A_wo: jax.Array,
    B_x: jax.Array,
    B_w1: jax.Array,
    B_w3: jax.Array,
    B_w2: jax.Array,
):
    B, Sq, D = A_x.shape
    _, hkv, sk, dh = A_k_cache.shape
    assert (B, Sq, hkv, dh) == (1, 1, HQ, DH)
    win = min(4096, max(256, sk // 4))
    ff = B_w1.shape[1]
    bf16, f32 = jnp.bfloat16, jnp.float32
    n_tail = len(_tail_chunks(ff)[0])

    kt = jnp.swapaxes(A_k_cache, 2, 3).reshape(HQ, DH, sk)
    vt = jnp.swapaxes(A_v_cache, 2, 3).reshape(HQ, DH, sk)
    x2 = A_x.reshape(1, D)
    wo3 = A_wo.reshape(HQ, DH, D)

    any_spec = pl.BlockSpec(memory_space=pl.ANY)
    out = pl.pallas_call(
        functools.partial(_kernel, win=win, sk=sk),
        out_shape=jax.ShapeDtypeStruct((1, D), A_x.dtype),
        in_specs=[any_spec] * 8,
        out_specs=pl.BlockSpec(memory_space=pltpu.VMEM),
        scratch_shapes=[
            pltpu.VMEM((1, D), bf16),
            pltpu.VMEM((HQ // 2, D, 2 * DH), bf16),
            pltpu.VMEM((HQ, DH, D), bf16),
            pltpu.VMEM((D, ff), bf16),
            pltpu.VMEM((D, ff), bf16),
            pltpu.VMEM((ff, D), bf16),
            pltpu.VMEM((NSLOT, DH, CW), bf16),
            pltpu.VMEM((win // CW, CW), f32),
            pltpu.VMEM((win // CW, CW), f32),
            pltpu.VMEM((1, D), f32),
            pltpu.VMEM((W2_VPU_ROWS * W2_VPU_CHUNKS, LANE), f32),
            pltpu.SemaphoreType.DMA((NSLOT * TPC,)),
            pltpu.SemaphoreType.DMA((4,)),
            pltpu.SemaphoreType.DMA((2,)),
            pltpu.SemaphoreType.DMA((5,)),
            pltpu.SemaphoreType.DMA((n_tail,)),
        ],
        compiler_params=pltpu.CompilerParams(
            vmem_limit_bytes=64 * 1024 * 1024,
            disable_bounds_checks=True,
            disable_semaphore_checks=True),
    )(x2, kt, vt, A_wq, wo3, B_w1, B_w3, B_w2)
    return out.reshape(B, Sq, D)
```
